```python
import jax
import jax.numpy as jnp

def _softmax(x, axis=-1):
    return jax.nn.softmax(x, axis=axis)
def _gelu(x):
    return jax.nn.gelu(x, approximate=True)
def _silu(x):
    return jax.nn.silu(x)
def _sigmoid(x):
    return jax.nn.sigmoid(x)
def _layernorm(x, axis=-1, eps=1e-5):
    m = jnp.mean(x, axis=axis, keepdims=True)
    v = jnp.var(x, axis=axis, keepdims=True)
    return (x - m) / jnp.sqrt(v + eps)
def _scatter_add(tgt, idx, src, axis=0):
    return tgt.at[idx].add(src)
def _segment_sum(src, seg, n):
    return jax.ops.segment_sum(src, seg, n)
class _Rng:
    def __init__(self, key):
        self._k = key
    def _next(self):
        self._k, sub = jax.random.split(self._k)
        return sub
    def normal(self, shape):
        return jax.random.normal(self._next(), shape, dtype=jnp.bfloat16)
    def randint(self, lo, hi, shape):
        return jax.random.randint(self._next(), shape, lo, hi, dtype=jnp.int32)
    def uniform(self, shape, lo=0.0, hi=1.0):
        return jax.random.uniform(self._next(), shape, jnp.bfloat16, lo, hi)
    def permutation(self, n):
        return jax.random.permutation(self._next(), n)


kernel_name = 'gated_mix__gqa_block_cached__dense_activation_relu__decode'

def _fwd_setup_inputs():
    _rng = _Rng(jax.random.key(int.from_bytes(__import__("os").urandom(4), "little")))
    _w = (lambda a: (lambda t: t.astype(jnp.bfloat16) if jnp.issubdtype(t.dtype, jnp.floating) else t)(jnp.asarray(a)))
    def _A_setup():
        B, Sq, D = 2, 1, 512
        Hq, Hkv, Sk, Dh = 32, 8, 8192, 128
        assert Hq % Hkv == 0, (Hq, Hkv)
        return {
            "x": _w((lambda *s: _rng.normal(s) * 0.05)(B, Sq, D)),
            "k_cache": _w((lambda *s: _rng.normal(s) * 0.05)(B, Hkv, Sk, Dh)),
            "v_cache": _w((lambda *s: _rng.normal(s) * 0.05)(B, Hkv, Sk, Dh)),
            "wq": _w((lambda *s: _rng.normal(s) * 0.05)(D, Hq * Dh) * (D ** -0.5)),
            "wo": _w((lambda *s: _rng.normal(s) * 0.05)(Hq * Dh, D) * ((Hq * Dh) ** -0.5)),
        }
    _A_in = _A_setup()

    def _B_setup():
        B, S, D, Dff = 2, 1, 512, 1792
        return {
            "x": _w((lambda *s: _rng.normal(s) * 0.05)(B, S, D)),
            "w1": _w((lambda *s: _rng.normal(s) * 0.05)(D, Dff)),
            "w2": _w((lambda *s: _rng.normal(s) * 0.05)(Dff, D)),
        }
    _B_in = _B_setup()

    return {
        "A_x": _A_in["x"],
        "A_k_cache": _A_in["k_cache"],
        "A_v_cache": _A_in["v_cache"],
        "A_wq": _A_in["wq"],
        "A_wo": _A_in["wo"],
        "B_x": _B_in["x"],
        "B_w1": _B_in["w1"],
        "B_w2": _B_in["w2"],
        "gate_w": _w((lambda *s: _rng.normal(s) * 0.05)(512)),
    }

def _fwd_reference(A_x, A_k_cache, A_v_cache, A_wq, A_wo, B_x, B_w1, B_w2, gate_w):
    def _A_ref(x, k_cache, v_cache, wq, wo):
        B, Sq, D = x.shape
        Hq, Dh = 32, 128
        Hkv = k_cache.shape[1]
        rep = Hq // Hkv
        q = (lambda x, *d: x.transpose(*d))((x @ wq).reshape(B, Sq, Hq, Dh), 0, 2, 1, 3)
        k = jnp.repeat(k_cache, rep, axis=1)
        v = jnp.repeat(v_cache, rep, axis=1)
        scores = jnp.einsum("bhqd,bhkd->bhqk", q, k) * (Dh ** -0.5)
        p = _softmax(scores, axis=-1)
        o = jnp.einsum("bhqk,bhkd->bhqd", p, v)
        return (lambda x, *d: x.transpose(*d))(o, 0, 2, 1, 3).reshape(B, Sq, Hq * Dh) @ wo

    def _B_ref(x, w1, w2):
        h = jnp.einsum("bsd,df->bsf", x, w1)
        zero = jnp.zeros_like(h)
        h = jnp.maximum(h, zero)
        return jnp.einsum("bsf,fd->bsd", h, w2)

    x = A_x
    g = _sigmoid((x * gate_w).sum(-1, keepdims=True))
    a = _A_ref(x, A_k_cache, A_v_cache, A_wq, A_wo)
    b = _B_ref(x, B_w1, B_w2)
    return g * a + (1 - g) * b


def setup_inputs():
    _inp = _fwd_setup_inputs()
    _gk = jax.random.fold_in(jax.random.key(int.from_bytes(__import__("os").urandom(4), "little")), 2**31 - 1)
    _shapes = [[2, 1, 512]]
    _dtypes = ['bfloat16']
    _gks = jax.random.split(_gk, len(_shapes))
    _gs = [jax.random.normal(k, s, dtype=jnp.dtype(d)) * 0.05 for k, s, d in zip(_gks, _shapes, _dtypes)]
    _inp["grad_out"] = _gs[0]
    return _inp

def reference(A_x, A_k_cache, A_v_cache, A_wq, A_wo, B_w1, B_w2, gate_w, B_x, grad_out):
    _const = dict(B_x=B_x)
    def _f(*_d):
        return _fwd_reference(**{'A_x': _d[0], 'A_k_cache': _d[1], 'A_v_cache': _d[2], 'A_wq': _d[3], 'A_wo': _d[4], 'B_w1': _d[5], 'B_w2': _d[6], 'gate_w': _d[7], **_const})
    _out, _vjp = jax.vjp(_f, A_x, A_k_cache, A_v_cache, A_wq, A_wo, B_w1, B_w2, gate_w)
    _grads = _vjp(grad_out)
    _out0 = jnp.asarray(_out)
    return (_out0, *[jnp.asarray(_g) for _g in _grads])
```

```python
import jax
import jax.numpy as jnp
from jax import lax
import jax.experimental.pallas as pl
import jax.experimental.pallas.tpu as pltpu

f32 = jnp.float32
bf16 = jnp.bfloat16

_NN = (((1,), (0,)), ((), ()))
_NT = (((1,), (1,)), ((), ()))

TRIG = 13
W2_TAIL = 384
NS = 8
WROWS = 64
QFILL = 80
QSTEP = 44
WS = 4
WPIECE = 16


def _dot(a, b, dims=_NN):
    return lax.dot_general(a, b, dims, preferred_element_type=f32)


@jax.jit
def pallas_gated_mix__gqa_block_cached__dense_activation_relu__decode_kernel(
    A_x: jax.Array,
    A_k_cache: jax.Array,
    A_v_cache: jax.Array,
    A_wq: jax.Array,
    A_wo: jax.Array,
    B_x: jax.Array,
    B_w1: jax.Array,
    B_w2: jax.Array,
    gate_w: jax.Array,
    grad_out: jax.Array,
):
    del B_x
    B, _, D = A_x.shape
    _, HKV, SK, DH = A_k_cache.shape
    HD = A_wq.shape[1]
    REP = HD // DH // HKV
    GW = REP * DH
    DFF = B_w1.shape[1]
    assert B == 2 and REP == 4 and DH == 128
    scale = DH ** -0.5
    NSTEP = B * HKV
    HALF = SK // 2
    kv_shape = (NSTEP * 2, HALF, DH)
    NJ = HALF // WROWS
    NKV = (kv_shape[0] // NS) * 2 * NJ
    W2_HEAD = DFF - W2_TAIL
    in_loop = QFILL + QSTEP * (NSTEP - 1 - TRIG)
    assert in_loop <= (2 * TRIG // NS) * 2 * NJ
    assert in_loop + 3 * QSTEP <= NKV

    def kernel(x_hbm, k_hbm, v_hbm, wq_hbm, wo_hbm, w1_hbm, w2_hbm, gw_hbm, go_hbm,
               out_hbm, dx_hbm, dk_hbm, dv_hbm, dwq_hbm, dwo_hbm, dw1_hbm, dw2_hbm, dgw_hbm,
               kbuf, vbuf, wq_b, wo_b, w1_b, w2_b, dwq_b, dwo_b, dw1_b, dw2_b,
               x_b, go_b, gw_b, out_b, dx_b, dgw_b,
               q_s, do_s, om_s, dqm_s, l_s, sem_w):
        cp = pltpu.make_async_copy

        def write_kv(lo, n):
            def body(t, c):
                r = lo + t
                idx = (pl.ds((r // (2 * NJ)) * NS, NS), pl.ds(pl.multiple_of((r % NJ) * WROWS, WROWS), WROWS))

                @pl.when((r // NJ) % 2 == 0)
                def _():
                    cp(kbuf.at[idx], dk_hbm.at[idx], sem_w).start()

                @pl.when((r // NJ) % 2 == 1)
                def _():
                    cp(vbuf.at[idx], dv_hbm.at[idx], sem_w).start()
                return c
            lax.fori_loop(0, n, body, 0)

        def token_rows():
            row16 = lax.broadcasted_iota(jnp.int32, (16, D), 0)
            xf = x_b[...].astype(f32)
            gof = go_b[...].astype(f32)
            gw = gw_b[...].astype(f32).reshape(1, D)
            x16 = jnp.where(row16 < 8, xf[0:1], xf[1:2])
            go16 = jnp.where(row16 < 8, gof[0:1], gof[1:2])
            g16 = jax.nn.sigmoid(jnp.sum(x16 * gw, axis=1, keepdims=True))
            return x16, go16, g16

        def read_phase(sem):
            rd_x = cp(x_hbm, x_b, sem.at[0])
            rd_go = cp(go_hbm, go_b, sem.at[1])
            rd_gw = cp(gw_hbm, gw_b, sem.at[2])
            rd_wq = cp(wq_hbm, wq_b, sem.at[3])
            rd_wo = cp(wo_hbm, wo_b, sem.at[4])
            rd_w1 = cp(w1_hbm, w1_b, sem.at[5])
            rd_w2a = cp(w2_hbm.at[pl.ds(0, W2_HEAD)], w2_b.at[pl.ds(0, W2_HEAD)], sem.at[6])
            rd_w2b = cp(w2_hbm.at[pl.ds(W2_HEAD, W2_TAIL)], w2_b.at[pl.ds(W2_HEAD, W2_TAIL)], sem.at[7])

            def rd_k(i):
                return cp(k_hbm.at[pl.ds(2 * i, 2)], kbuf.at[pl.ds(2 * i, 2)], sem.at[8 + 2 * i])

            def rd_v(i):
                return cp(v_hbm.at[pl.ds(2 * i, 2)], vbuf.at[pl.ds(2 * i, 2)], sem.at[9 + 2 * i])

            for c in (rd_x, rd_go, rd_gw, rd_wq, rd_wo):
                c.start()
            for i in range(NSTEP):
                rd_k(i).start()
                rd_v(i).start()
            for c in (rd_w1, rd_w2a, rd_w2b):
                c.start()

            for c in (rd_x, rd_go, rd_gw):
                c.wait()
            x16, go16, g16 = token_rows()
            rd_wq.wait()
            q_s[...] = _dot(x16.astype(bf16), wq_b[...])
            rd_wo.wait()
            do_s[...] = _dot((g16 * go16).astype(bf16), wo_b[...], _NT)

            row8 = lax.broadcasted_iota(jnp.int32, (8, DH), 0)

            def per_head_rows(blk):
                out = blk[:, 0:DH]
                for j in range(1, REP):
                    out = jnp.where(row8 % REP == j, blk[:, j * DH:(j + 1) * DH], out)
                return out

            def step(i, carry):
                @pl.when(i == TRIG)
                def _():
                    rd_w1.wait()
                    rd_w2a.wait()
                    write_kv(0, QFILL)

                @pl.when(i > TRIG)
                def _():
                    write_kv(QFILL + QSTEP * (i - TRIG - 1), QSTEP)

                rows = pl.ds(pl.multiple_of((i // HKV) * 8, 8), 8)
                cols = pl.ds(pl.multiple_of((i % HKV) * GW, GW), GW)
                q8 = per_head_rows(q_s[rows, cols])
                do8 = per_head_rows(do_s[rows, cols])
                do_hi = jnp.where(row8 >= REP, do8, 0.0).astype(bf16)
                w3 = jnp.concatenate(
                    [jnp.where(row8 < REP, do8, 0.0), jnp.where(row8 >= REP, q8, 0.0)], axis=1).astype(bf16)
                rd_k(i).wait()
                rd_v(i).wait()

                k_all = kbuf[pl.ds(2 * i, 2)].reshape(SK, DH)
                v_all = vbuf[pl.ds(2 * i, 2)].reshape(SK, DH)
                s = _dot(q8.astype(bf16), k_all, _NT) * scale
                dp = _dot(do_hi, v_all, _NT)
                e = jnp.exp(s - jnp.max(s, axis=1, keepdims=True))
                p = e * (1.0 / jnp.sum(e, axis=1, keepdims=True))
                delta = jnp.sum(p * dp, axis=1, keepdims=True)
                rowk = lax.broadcasted_iota(jnp.int32, (8, SK), 0)
                l_s[...] = p * jnp.where(rowk < REP, 1.0, (dp - delta) * scale)

                def second_pass(c, acc):
                    lc = l_s[:, pl.ds(pl.multiple_of(c * HALF, HALF), HALF)]
                    lb = lc.astype(bf16)
                    o = _dot(lb, vbuf[2 * i + c])
                    dq = _dot(lb, kbuf[2 * i + c])
                    r = _dot(lc.T.astype(bf16), w3)
                    vbuf[2 * i + c] = r[:, :DH].astype(bf16)
                    kbuf[2 * i + c] = r[:, DH:].astype(bf16)
                    return acc[0] + o, acc[1] + dq
                z = jnp.zeros((8, DH), f32)
                o8, dq8 = lax.fori_loop(0, 2, second_pass, (z, z))
                om_s[rows, cols] = jnp.concatenate(
                    [jnp.where(row8 == j, o8, 0.0) for j in range(REP)], axis=1)
                dqm_s[rows, cols] = jnp.concatenate(
                    [jnp.where(row8 == REP + j, dq8, 0.0) for j in range(REP)], axis=1)
                return carry

            lax.fori_loop(0, NSTEP, step, 0)
            rd_w2b.wait()

        pl.run_scoped(read_phase, pltpu.SemaphoreType.DMA((8 + 2 * NSTEP,)))

        write_kv(in_loop, QSTEP)
        x16, go16, g16 = token_rows()
        x16b = x16.astype(bf16)
        x16t = x16.T.astype(bf16)
        da16b = (g16 * go16).astype(bf16)
        db16b = ((1.0 - g16) * go16).astype(bf16)
        hpre = _dot(x16b, w1_b[...])
        hact = jnp.maximum(hpre, 0.0)
        mlp16 = _dot(hact.astype(bf16), w2_b[...])
        slope = jnp.where(hpre > 0.0, 1.0, jnp.where(hpre == 0.0, 0.5, 0.0))
        dh = _dot(db16b, w2_b[...], _NT) * slope
        dxm16 = _dot(dh.astype(bf16), w1_b[...], _NT)
        lead = lax.broadcasted_iota(jnp.int32, (16, DFF), 0) % 8 == 0
        dw1_b[...] = _dot(x16t, jnp.where(lead, dh, 0.0).astype(bf16)).astype(bf16).reshape(dw1_b.shape)
        dw2_b[...] = _dot(jnp.where(lead, hact, 0.0).T.astype(bf16), db16b).astype(bf16).reshape(dw2_b.shape)
        write_kv(in_loop + QSTEP, QSTEP)

        dqmb = dqm_s[...].astype(bf16)
        a16 = _dot(om_s[...].astype(bf16), wo_b[...])
        dxq16 = _dot(dqmb, wq_b[...], _NT)
        row2 = lax.broadcasted_iota(jnp.int32, (B, D), 0)

        def fold(m):
            return jnp.where(row2 == 0, jnp.sum(m[0:8], axis=0, keepdims=True),
                             jnp.sum(m[8:16], axis=0, keepdims=True))

        def pick(m):
            return jnp.where(row2 == 0, m[0:1], m[8:9])

        xf = x_b[...].astype(f32)
        gof = go_b[...].astype(f32)
        gw = gw_b[...].astype(f32).reshape(1, D)
        a2 = fold(a16)
        m2 = pick(mlp16)
        g2 = jax.nn.sigmoid(jnp.sum(xf * gw, axis=1, keepdims=True))
        out_b[...] = (g2 * a2 + (1.0 - g2) * m2).astype(bf16)
        dz = jnp.sum(gof * (a2 - m2), axis=1, keepdims=True) * g2 * (1.0 - g2)
        dx_b[...] = (fold(dxq16) + pick(dxm16) + dz * gw).astype(bf16)
        dgw_b[...] = jnp.sum(dz * xf, axis=0).astype(bf16)
        for src, dst in ((out_b, out_hbm), (dx_b, dx_hbm), (dgw_b, dgw_hbm)):
            cp(src, dst, sem_w).start()
        dwq_b[...] = _dot(x16t, dqmb).astype(bf16).reshape(dwq_b.shape)
        write_kv(in_loop + 2 * QSTEP, QSTEP)
        dwo_b[...] = _dot(om_s[...].T.astype(bf16), da16b).astype(bf16).reshape(dwo_b.shape)
        write_kv(in_loop + 3 * QSTEP, NKV - in_loop - 3 * QSTEP)

        def pieces(buf, dst):
            _, nrow, ncol = buf.shape
            rstep = max(8, WPIECE * 1024 // (ncol * 2) // 8 * 8)
            cstep = ncol // max(1, rstep * ncol * 2 // (WPIECE * 1024))
            assert nrow % rstep == 0 and ncol % cstep == 0 and cstep % 128 == 0
            return [(buf, dst, (slice(None), pl.ds(r0, rstep), pl.ds(c0, cstep)))
                    for r0 in range(0, nrow, rstep) for c0 in range(0, ncol, cstep)]

        def merge(*lists):
            keyed = [((n + 0.5) / len(l), k, d) for k, l in enumerate(lists) for n, d in enumerate(l)]
            return [d for _, _, d in sorted(keyed, key=lambda t: t[:2])]

        for buf, dst, idx in (merge(pieces(dw1_b, dw1_hbm), pieces(dw2_b, dw2_hbm))
                              + merge(pieces(dwq_b, dwq_hbm), pieces(dwo_b, dwo_hbm))):
            cp(buf.at[idx], dst.at[idx], sem_w).start()

        for src, dst in ((out_b, out_hbm), (dx_b, dx_hbm), (dgw_b, dgw_hbm), (dw1_b, dw1_hbm),
                         (dw2_b, dw2_hbm), (dwq_b, dwq_hbm), (dwo_b, dwo_hbm), (kbuf, dk_hbm), (vbuf, dv_hbm)):
            cp(src, dst, sem_w).wait()

    hbm = pl.BlockSpec(memory_space=pltpu.MemorySpace.HBM)
    sds = jax.ShapeDtypeStruct
    weights = (A_wq, A_wo, B_w1, B_w2)
    wsplit = [(WS, w.shape[0] // WS, w.shape[1]) for w in weights]
    outs = pl.pallas_call(
        kernel,
        in_specs=[hbm] * 9,
        out_specs=[hbm] * 9,
        out_shape=[sds((B, D), bf16), sds((B, D), bf16), sds(kv_shape, bf16), sds(kv_shape, bf16)]
        + [sds(s, bf16) for s in wsplit] + [sds(gate_w.shape, bf16)],
        scratch_shapes=[pltpu.VMEM(kv_shape, bf16)] * 2
        + [pltpu.VMEM(w.shape, bf16) for w in weights]
        + [pltpu.VMEM(s, bf16) for s in wsplit]
        + [pltpu.VMEM((B, D), bf16), pltpu.VMEM((B, D), bf16), pltpu.VMEM((D,), bf16)] * 2
        + [pltpu.VMEM((16, HD), f32)] * 4
        + [pltpu.VMEM((8, SK), f32), pltpu.SemaphoreType.DMA(())],
        compiler_params=pltpu.CompilerParams(vmem_limit_bytes=110 * 1024 * 1024),
    )(A_x.reshape(B, D), A_k_cache.reshape(kv_shape), A_v_cache.reshape(kv_shape), A_wq, A_wo,
      B_w1, B_w2, gate_w, grad_out.reshape(B, D))
    return (outs[0].reshape(A_x.shape), outs[1].reshape(A_x.shape),
            outs[2].reshape(A_k_cache.shape), outs[3].reshape(A_v_cache.shape),
            *[o.reshape(w.shape) for o, w in zip(outs[4:8], weights)], outs[8])
```

```python
import jax
import jax.numpy as jnp
from jax import lax
import jax.experimental.pallas as pl
import jax.experimental.pallas.tpu as pltpu

f32 = jnp.float32
bf16 = jnp.bfloat16

_NN = (((1,), (0,)), ((), ()))
_NT = (((1,), (1,)), ((), ()))

TRIG = 13
W2_TAIL = 384
NS = 8
WROWS = 64
QFILL = 80
QSTEP = 44
WS = 4
WPIECE = 16


def _dot(a, b, dims=_NN):
    return lax.dot_general(a, b, dims, preferred_element_type=f32)


@jax.jit
def pallas_gated_mix__gqa_block_cached__dense_activation_relu__decode_kernel(
    A_x: jax.Array,
    A_k_cache: jax.Array,
    A_v_cache: jax.Array,
    A_wq: jax.Array,
    A_wo: jax.Array,
    B_x: jax.Array,
    B_w1: jax.Array,
    B_w2: jax.Array,
    gate_w: jax.Array,
    grad_out: jax.Array,
):
    del B_x
    B, _, D = A_x.shape
    _, HKV, SK, DH = A_k_cache.shape
    HD = A_wq.shape[1]
    REP = HD // DH // HKV
    GW = REP * DH
    DFF = B_w1.shape[1]
    assert B == 2 and REP == 4 and DH == 128
    scale = DH ** -0.5
    NSTEP = B * HKV
    HALF = SK // 2
    kv_shape = (NSTEP * 2, HALF, DH)
    NJ = HALF // WROWS
    NKV = (kv_shape[0] // NS) * 2 * NJ
    W2_HEAD = DFF - W2_TAIL
    in_loop = QFILL + QSTEP * (NSTEP - 1 - TRIG)
    assert in_loop <= (2 * TRIG // NS) * 2 * NJ
    assert in_loop + 3 * QSTEP <= NKV

    def kernel(x_hbm, k_hbm, v_hbm, wq_hbm, wo_hbm, w1_hbm, w2_hbm, gw_hbm, go_hbm,
               out_hbm, dx_hbm, dk_hbm, dv_hbm, dwq_hbm, dwo_hbm, dw1_hbm, dw2_hbm, dgw_hbm,
               kbuf, vbuf, wq_b, wo_b, w1_b, w2_b, dwq_b, dwo_b, dw1_b, dw2_b,
               x_b, go_b, gw_b, out_b, dx_b, dgw_b,
               q_s, do_s, om_s, dqm_s, l_s, sem_w):
        cp = pltpu.make_async_copy

        def write_kv(lo, n):
            def body(t, c):
                r = lo + t
                idx = (pl.ds((r // (2 * NJ)) * NS, NS), pl.ds(pl.multiple_of((r % NJ) * WROWS, WROWS), WROWS))

                @pl.when((r // NJ) % 2 == 0)
                def _():
                    cp(kbuf.at[idx], dk_hbm.at[idx], sem_w).start()

                @pl.when((r // NJ) % 2 == 1)
                def _():
                    cp(vbuf.at[idx], dv_hbm.at[idx], sem_w).start()
                return c
            lax.fori_loop(0, n, body, 0)

        def token_rows():
            row16 = lax.broadcasted_iota(jnp.int32, (16, D), 0)
            xf = x_b[...].astype(f32)
            gof = go_b[...].astype(f32)
            gw = gw_b[...].astype(f32).reshape(1, D)
            x16 = jnp.where(row16 < 8, xf[0:1], xf[1:2])
            go16 = jnp.where(row16 < 8, gof[0:1], gof[1:2])
            g16 = jax.nn.sigmoid(jnp.sum(x16 * gw, axis=1, keepdims=True))
            return x16, go16, g16

        def read_phase(sem):
            rd_x = cp(x_hbm, x_b, sem.at[0])
            rd_go = cp(go_hbm, go_b, sem.at[1])
            rd_gw = cp(gw_hbm, gw_b, sem.at[2])
            rd_wq = cp(wq_hbm, wq_b, sem.at[3])
            rd_wo = cp(wo_hbm, wo_b, sem.at[4])
            rd_w1 = cp(w1_hbm, w1_b, sem.at[5])
            rd_w2a = cp(w2_hbm.at[pl.ds(0, W2_HEAD)], w2_b.at[pl.ds(0, W2_HEAD)], sem.at[6])
            rd_w2b = cp(w2_hbm.at[pl.ds(W2_HEAD, W2_TAIL)], w2_b.at[pl.ds(W2_HEAD, W2_TAIL)], sem.at[7])

            def rd_k(i):
                return cp(k_hbm.at[pl.ds(2 * i, 2)], kbuf.at[pl.ds(2 * i, 2)], sem.at[8 + 2 * i])

            def rd_v(i):
                return cp(v_hbm.at[pl.ds(2 * i, 2)], vbuf.at[pl.ds(2 * i, 2)], sem.at[9 + 2 * i])

            for c in (rd_x, rd_go, rd_gw, rd_wq, rd_wo):
                c.start()
            for i in range(NSTEP):
                rd_k(i).start()
                rd_v(i).start()
            for c in (rd_w1, rd_w2a, rd_w2b):
                c.start()

            for c in (rd_x, rd_go, rd_gw):
                c.wait()
            x16, go16, g16 = token_rows()
            rd_wq.wait()
            q_s[...] = _dot(x16.astype(bf16), wq_b[...])
            rd_wo.wait()
            do_s[...] = _dot((g16 * go16).astype(bf16), wo_b[...], _NT)

            row8 = lax.broadcasted_iota(jnp.int32, (8, DH), 0)

            def per_head_rows(blk):
                out = blk[:, 0:DH]
                for j in range(1, REP):
                    out = jnp.where(row8 % REP == j, blk[:, j * DH:(j + 1) * DH], out)
                return out

            def step(i, carry):
                @pl.when(i == TRIG)
                def _():
                    rd_w1.wait()
                    rd_w2a.wait()
                    write_kv(0, QFILL)

                @pl.when(i > TRIG)
                def _():
                    write_kv(QFILL + QSTEP * (i - TRIG - 1), QSTEP)

                rows = pl.ds(pl.multiple_of((i // HKV) * 8, 8), 8)
                cols = pl.ds(pl.multiple_of((i % HKV) * GW, GW), GW)
                q8 = per_head_rows(q_s[rows, cols])
                do8 = per_head_rows(do_s[rows, cols])
                do_hi = jnp.where(row8 >= REP, do8, 0.0).astype(bf16)
                w3 = jnp.concatenate(
                    [jnp.where(row8 < REP, do8, 0.0), jnp.where(row8 >= REP, q8, 0.0)], axis=1).astype(bf16)
                rd_k(i).wait()
                rd_v(i).wait()

                k_all = kbuf[pl.ds(2 * i, 2)].reshape(SK, DH)
                v_all = vbuf[pl.ds(2 * i, 2)].reshape(SK, DH)
                s = _dot(q8.astype(bf16), k_all, _NT) * scale
                dp = _dot(do_hi, v_all, _NT)
                e = jnp.exp(s - jnp.max(s, axis=1, keepdims=True))
                p = e * (1.0 / jnp.sum(e, axis=1, keepdims=True))
                delta = jnp.sum(p * dp, axis=1, keepdims=True)
                rowk = lax.broadcasted_iota(jnp.int32, (8, SK), 0)
                l_s[...] = p * jnp.where(rowk < REP, 1.0, (dp - delta) * scale)

                def second_pass(c, acc):
                    lc = l_s[:, pl.ds(pl.multiple_of(c * HALF, HALF), HALF)]
                    lb = lc.astype(bf16)
                    o = _dot(lb, vbuf[2 * i + c])
                    dq = _dot(lb, kbuf[2 * i + c])
                    r = _dot(lc.T.astype(bf16), w3)
                    vbuf[2 * i + c] = r[:, :DH].astype(bf16)
                    kbuf[2 * i + c] = r[:, DH:].astype(bf16)
                    return acc[0] + o, acc[1] + dq
                z = jnp.zeros((8, DH), f32)
                o8, dq8 = lax.fori_loop(0, 2, second_pass, (z, z))
                om_s[rows, cols] = jnp.concatenate(
                    [jnp.where(row8 == j, o8, 0.0) for j in range(REP)], axis=1)
                dqm_s[rows, cols] = jnp.concatenate(
                    [jnp.where(row8 == REP + j, dq8, 0.0) for j in range(REP)], axis=1)
                return carry

            lax.fori_loop(0, NSTEP, step, 0)
            rd_w2b.wait()

        pl.run_scoped(read_phase, pltpu.SemaphoreType.DMA((8 + 2 * NSTEP,)))

        write_kv(in_loop, QSTEP)
        x16, go16, g16 = token_rows()
        x16b = x16.astype(bf16)
        x16t = x16.T.astype(bf16)
        da16b = (g16 * go16).astype(bf16)
        db16b = ((1.0 - g16) * go16).astype(bf16)
        hpre = _dot(x16b, w1_b[...])
        hact = jnp.maximum(hpre, 0.0)
        mlp16 = _dot(hact.astype(bf16), w2_b[...])
        slope = jnp.where(hpre > 0.0, 1.0, jnp.where(hpre == 0.0, 0.5, 0.0))
        dh = _dot(db16b, w2_b[...], _NT) * slope
        dxm16 = _dot(dh.astype(bf16), w1_b[...], _NT)
        lead = lax.broadcasted_iota(jnp.int32, (16, DFF), 0) % 8 == 0
        dw1_b[...] = _dot(x16t, jnp.where(lead, dh, 0.0).astype(bf16)).astype(bf16).reshape(dw1_b.shape)
        dw2_b[...] = _dot(jnp.where(lead, hact, 0.0).T.astype(bf16), db16b).astype(bf16).reshape(dw2_b.shape)
        write_kv(in_loop + QSTEP, QSTEP)

        dqmb = dqm_s[...].astype(bf16)
        a16 = _dot(om_s[...].astype(bf16), wo_b[...])
        dxq16 = _dot(dqmb, wq_b[...], _NT)
        row2 = lax.broadcasted_iota(jnp.int32, (B, D), 0)

        def fold(m):
            return jnp.where(row2 == 0, jnp.sum(m[0:8], axis=0, keepdims=True),
                             jnp.sum(m[8:16], axis=0, keepdims=True))

        def pick(m):
            return jnp.where(row2 == 0, m[0:1], m[8:9])

        xf = x_b[...].astype(f32)
        gof = go_b[...].astype(f32)
        gw = gw_b[...].astype(f32).reshape(1, D)
        a2 = fold(a16)
        m2 = pick(mlp16)
        g2 = jax.nn.sigmoid(jnp.sum(xf * gw, axis=1, keepdims=True))
        out_b[...] = (g2 * a2 + (1.0 - g2) * m2).astype(bf16)
        dz = jnp.sum(gof * (a2 - m2), axis=1, keepdims=True) * g2 * (1.0 - g2)
        dx_b[...] = (fold(dxq16) + pick(dxm16) + dz * gw).astype(bf16)
        dgw_b[...] = jnp.sum(dz * xf, axis=0).astype(bf16)
        for src, dst in ((out_b, out_hbm), (dx_b, dx_hbm), (dgw_b, dgw_hbm)):
            cp(src, dst, sem_w).start()
        dwq_b[...] = _dot(x16t, dqmb).astype(bf16).reshape(dwq_b.shape)
        write_kv(in_loop + 2 * QSTEP, QSTEP)
        dwo_b[...] = _dot(om_s[...].T.astype(bf16), da16b).astype(bf16).reshape(dwo_b.shape)
        write_kv(in_loop + 3 * QSTEP, NKV - in_loop - 3 * QSTEP)

        def pieces(buf, dst):
            _, nblk, nrow, ncol = buf.shape
            cstep = ncol // max(1, nrow * ncol * 2 // (WPIECE * 1024))
            assert ncol % cstep == 0 and cstep % 128 == 0
            return [(buf, dst, (slice(None), r, slice(None), pl.ds(c0, cstep)))
                    for r in range(nblk) for c0 in range(0, ncol, cstep)]

        def merge(*lists):
            keyed = [((n + 0.5) / len(l), k, d) for k, l in enumerate(lists) for n, d in enumerate(l)]
            return [d for _, _, d in sorted(keyed, key=lambda t: t[:2])]

        for buf, dst, idx in (merge(pieces(dw1_b, dw1_hbm), pieces(dw2_b, dw2_hbm))
                              + merge(pieces(dwq_b, dwq_hbm), pieces(dwo_b, dwo_hbm))):
            cp(buf.at[idx], dst.at[idx], sem_w).start()

        for src, dst in ((out_b, out_hbm), (dx_b, dx_hbm), (dgw_b, dgw_hbm), (dw1_b, dw1_hbm),
                         (dw2_b, dw2_hbm), (dwq_b, dwq_hbm), (dwo_b, dwo_hbm), (kbuf, dk_hbm), (vbuf, dv_hbm)):
            cp(src, dst, sem_w).wait()

    hbm = pl.BlockSpec(memory_space=pltpu.MemorySpace.HBM)
    sds = jax.ShapeDtypeStruct
    weights = (A_wq, A_wo, B_w1, B_w2)
    wrows = [max(8, WPIECE * 1024 // (w.shape[1] * 2) // 8 * 8) for w in weights]
    wsplit = [(WS, w.shape[0] // WS // n, n, w.shape[1]) for w, n in zip(weights, wrows)]
    outs = pl.pallas_call(
        kernel,
        in_specs=[hbm] * 9,
        out_specs=[hbm] * 9,
        out_shape=[sds((B, D), bf16), sds((B, D), bf16), sds(kv_shape, bf16), sds(kv_shape, bf16)]
        + [sds(s, bf16) for s in wsplit] + [sds(gate_w.shape, bf16)],
        scratch_shapes=[pltpu.VMEM(kv_shape, bf16)] * 2
        + [pltpu.VMEM(w.shape, bf16) for w in weights]
        + [pltpu.VMEM(s, bf16) for s in wsplit]
        + [pltpu.VMEM((B, D), bf16), pltpu.VMEM((B, D), bf16), pltpu.VMEM((D,), bf16)] * 2
        + [pltpu.VMEM((16, HD), f32)] * 4
        + [pltpu.VMEM((8, SK), f32), pltpu.SemaphoreType.DMA(())],
        compiler_params=pltpu.CompilerParams(vmem_limit_bytes=110 * 1024 * 1024),
    )(A_x.reshape(B, D), A_k_cache.reshape(kv_shape), A_v_cache.reshape(kv_shape), A_wq, A_wo,
      B_w1, B_w2, gate_w, grad_out.reshape(B, D))
    return (outs[0].reshape(A_x.shape), outs[1].reshape(A_x.shape),
            outs[2].reshape(A_k_cache.shape), outs[3].reshape(A_v_cache.shape),
            *[o.reshape(w.shape) for o, w in zip(outs[4:8], weights)], outs[8])
```

```python
import functools

import jax
import jax.numpy as jnp
from jax import lax
import jax.experimental.pallas as pl
import jax.experimental.pallas.tpu as pltpu

f32 = jnp.float32
bf16 = jnp.bfloat16

_NN = (((1,), (0,)), ((), ()))
_NT = (((1,), (1,)), ((), ()))

TRIG = 13
W2_TAIL = 384
NS = 8
WROWS = 64
WS = 4
WPIECE = 16


def _dot(a, b, dims=_NN):
    return lax.dot_general(a, b, dims, preferred_element_type=f32)


@jax.jit
def pallas_gated_mix__gqa_block_cached__dense_activation_relu__decode_kernel(
    A_x: jax.Array,
    A_k_cache: jax.Array,
    A_v_cache: jax.Array,
    A_wq: jax.Array,
    A_wo: jax.Array,
    B_x: jax.Array,
    B_w1: jax.Array,
    B_w2: jax.Array,
    gate_w: jax.Array,
    grad_out: jax.Array,
):
    del B_x
    B, _, D = A_x.shape
    _, HKV, SK, DH = A_k_cache.shape
    HD = A_wq.shape[1]
    REP = HD // DH // HKV
    GW = REP * DH
    DFF = B_w1.shape[1]
    assert B == 2 and REP == 4 and DH == 128
    scale = DH ** -0.5
    NSTEP = B * HKV
    HALF = SK // 2
    kv_shape = (NSTEP * 2, HALF, DH)
    NJ = HALF // WROWS
    NBLK = (kv_shape[0] // NS) * 2
    W2_HEAD = DFF - W2_TAIL
    in_loop = NSTEP - TRIG
    assert in_loop <= (2 * TRIG // NS) * 2
    assert in_loop + 3 <= NBLK
    assert HALF % WROWS == 0 and kv_shape[0] % NS == 0 and W2_HEAD % 16 == 0

    def kernel(x_hbm, k_hbm, v_hbm, wq_hbm, wo_hbm, w1_hbm, w2_hbm, gw_hbm, go_hbm,
               out_hbm, dx_hbm, dk_hbm, dv_hbm, dwq_hbm, dwo_hbm, dw1_hbm, dw2_hbm, dgw_hbm,
               kbuf, vbuf, wq_b, wo_b, w1_b, w2_b, dwq_b, dwo_b, dw1_b, dw2_b,
               x_b, go_b, gw_b, out_b, dx_b, dgw_b,
               q_s, do_s, om_s, dqm_s, l_s, sem_w):
        cp = pltpu.make_async_copy

        def write_kv(blk):
            buf, dst = ((kbuf, dk_hbm), (vbuf, dv_hbm))[blk % 2]
            heads = pl.ds((blk // 2) * NS, NS)

            def body(j, c):
                idx = (heads, pl.ds(pl.multiple_of(j * WROWS, WROWS), WROWS))
                cp(buf.at[idx], dst.at[idx], sem_w).start()
                return c
            lax.fori_loop(0, NJ, body, 0)

        def token_rows():
            row16 = lax.broadcasted_iota(jnp.int32, (16, D), 0)
            xf = x_b[...].astype(f32)
            gof = go_b[...].astype(f32)
            gw = gw_b[...].astype(f32).reshape(1, D)
            x16 = jnp.where(row16 < 8, xf[0:1], xf[1:2])
            go16 = jnp.where(row16 < 8, gof[0:1], gof[1:2])
            g16 = jax.nn.sigmoid(jnp.sum(x16 * gw, axis=1, keepdims=True))
            return x16, go16, g16

        def read_phase(sem):
            rd_x = cp(x_hbm, x_b, sem.at[0])
            rd_go = cp(go_hbm, go_b, sem.at[1])
            rd_gw = cp(gw_hbm, gw_b, sem.at[2])
            rd_wq = cp(wq_hbm, wq_b, sem.at[3])
            rd_wo = cp(wo_hbm, wo_b, sem.at[4])
            rd_w1 = cp(w1_hbm, w1_b, sem.at[5])
            rd_w2a = cp(w2_hbm.at[pl.ds(0, W2_HEAD)], w2_b.at[pl.ds(0, W2_HEAD)], sem.at[6])
            rd_w2b = cp(w2_hbm.at[pl.ds(W2_HEAD, W2_TAIL)], w2_b.at[pl.ds(W2_HEAD, W2_TAIL)], sem.at[7])

            def rd_k(i):
                return cp(k_hbm.at[pl.ds(2 * i, 2)], kbuf.at[pl.ds(2 * i, 2)], sem.at[8 + 2 * i])

            def rd_v(i):
                return cp(v_hbm.at[pl.ds(2 * i, 2)], vbuf.at[pl.ds(2 * i, 2)], sem.at[9 + 2 * i])

            for c in (rd_x, rd_go, rd_gw, rd_wq, rd_wo):
                c.start()
            for i in range(NSTEP):
                rd_k(i).start()
                rd_v(i).start()
            for c in (rd_w1, rd_w2a, rd_w2b):
                c.start()

            for c in (rd_x, rd_go, rd_gw):
                c.wait()
            x16, go16, g16 = token_rows()
            rd_wq.wait()
            q_s[...] = _dot(x16.astype(bf16), wq_b[...])
            rd_wo.wait()
            do_s[...] = _dot((g16 * go16).astype(bf16), wo_b[...], _NT)

            row8 = lax.broadcasted_iota(jnp.int32, (8, DH), 0)

            def per_head_rows(blk):
                out = blk[:, 0:DH]
                for j in range(1, REP):
                    out = jnp.where(row8 % REP == j, blk[:, j * DH:(j + 1) * DH], out)
                return out

            def step(i, carry):
                @pl.when(i == TRIG)
                def _():
                    rd_w1.wait()
                    rd_w2a.wait()

                for blk in range(in_loop):
                    pl.when(i == TRIG + blk)(functools.partial(write_kv, blk))

                rows = pl.ds(pl.multiple_of((i // HKV) * 8, 8), 8)
                cols = pl.ds(pl.multiple_of((i % HKV) * GW, GW), GW)
                q8 = per_head_rows(q_s[rows, cols])
                do8 = per_head_rows(do_s[rows, cols])
                do_hi = jnp.where(row8 >= REP, do8, 0.0).astype(bf16)
                w3 = jnp.concatenate(
                    [jnp.where(row8 < REP, do8, 0.0), jnp.where(row8 >= REP, q8, 0.0)], axis=1).astype(bf16)
                rd_k(i).wait()
                rd_v(i).wait()

                k_all = kbuf[pl.ds(2 * i, 2)].reshape(SK, DH)
                v_all = vbuf[pl.ds(2 * i, 2)].reshape(SK, DH)
                s = _dot(q8.astype(bf16), k_all, _NT) * scale
                dp = _dot(do_hi, v_all, _NT)
                e = jnp.exp(s - jnp.max(s, axis=1, keepdims=True))
                p = e * (1.0 / jnp.sum(e, axis=1, keepdims=True))
                delta = jnp.sum(p * dp, axis=1, keepdims=True)
                rowk = lax.broadcasted_iota(jnp.int32, (8, SK), 0)
                l_s[...] = p * jnp.where(rowk < REP, 1.0, (dp - delta) * scale)

                def second_pass(c, acc):
                    lc = l_s[:, pl.ds(pl.multiple_of(c * HALF, HALF), HALF)]
                    lb = lc.astype(bf16)
                    o = _dot(lb, vbuf[2 * i + c])
                    dq = _dot(lb, kbuf[2 * i + c])
                    r = _dot(lc.T.astype(bf16), w3)
                    vbuf[2 * i + c] = r[:, :DH].astype(bf16)
                    kbuf[2 * i + c] = r[:, DH:].astype(bf16)
                    return acc[0] + o, acc[1] + dq
                z = jnp.zeros((8, DH), f32)
                o8, dq8 = lax.fori_loop(0, 2, second_pass, (z, z))
                om_s[rows, cols] = jnp.concatenate(
                    [jnp.where(row8 == j, o8, 0.0) for j in range(REP)], axis=1)
                dqm_s[rows, cols] = jnp.concatenate(
                    [jnp.where(row8 == REP + j, dq8, 0.0) for j in range(REP)], axis=1)
                return carry

            lax.fori_loop(0, NSTEP, step, 0)
            rd_w2b.wait()

        pl.run_scoped(read_phase, pltpu.SemaphoreType.DMA((8 + 2 * NSTEP,)))

        write_kv(in_loop)
        x16, go16, g16 = token_rows()
        x16b = x16.astype(bf16)
        x16t = x16.T.astype(bf16)
        da16b = (g16 * go16).astype(bf16)
        db16b = ((1.0 - g16) * go16).astype(bf16)
        hpre = _dot(x16b, w1_b[...])
        hact = jnp.maximum(hpre, 0.0)
        mlp16 = _dot(hact.astype(bf16), w2_b[...])
        slope = jnp.where(hpre > 0.0, 1.0, jnp.where(hpre == 0.0, 0.5, 0.0))
        dh = _dot(db16b, w2_b[...], _NT) * slope
        dxm16 = _dot(dh.astype(bf16), w1_b[...], _NT)
        lead = lax.broadcasted_iota(jnp.int32, (16, DFF), 0) % 8 == 0
        dw1_b[...] = _dot(x16t, jnp.where(lead, dh, 0.0).astype(bf16)).astype(bf16).reshape(dw1_b.shape)
        dw2_b[...] = _dot(jnp.where(lead, hact, 0.0).T.astype(bf16), db16b).astype(bf16).reshape(dw2_b.shape)
        write_kv(in_loop + 1)

        dqmb = dqm_s[...].astype(bf16)
        a16 = _dot(om_s[...].astype(bf16), wo_b[...])
        dxq16 = _dot(dqmb, wq_b[...], _NT)
        row2 = lax.broadcasted_iota(jnp.int32, (B, D), 0)

        def fold(m):
            return jnp.where(row2 == 0, jnp.sum(m[0:8], axis=0, keepdims=True),
                             jnp.sum(m[8:16], axis=0, keepdims=True))

        def pick(m):
            return jnp.where(row2 == 0, m[0:1], m[8:9])

        xf = x_b[...].astype(f32)
        gof = go_b[...].astype(f32)
        gw = gw_b[...].astype(f32).reshape(1, D)
        a2 = fold(a16)
        m2 = pick(mlp16)
        g2 = jax.nn.sigmoid(jnp.sum(xf * gw, axis=1, keepdims=True))
        out_b[...] = (g2 * a2 + (1.0 - g2) * m2).astype(bf16)
        dz = jnp.sum(gof * (a2 - m2), axis=1, keepdims=True) * g2 * (1.0 - g2)
        dx_b[...] = (fold(dxq16) + pick(dxm16) + dz * gw).astype(bf16)
        dgw_b[...] = jnp.sum(dz * xf, axis=0).astype(bf16)
        for src, dst in ((out_b, out_hbm), (dx_b, dx_hbm), (dgw_b, dgw_hbm)):
            cp(src, dst, sem_w).start()
        dwq_b[...] = _dot(x16t, dqmb).astype(bf16).reshape(dwq_b.shape)
        write_kv(in_loop + 2)
        dwo_b[...] = _dot(om_s[...].T.astype(bf16), da16b).astype(bf16).reshape(dwo_b.shape)
        for blk in range(in_loop + 3, NBLK):
            write_kv(blk)

        def pieces(buf, dst):
            _, nblk, nrow, ncol = buf.shape
            cstep = ncol // max(1, nrow * ncol * 2 // (WPIECE * 1024))
            assert ncol % cstep == 0 and cstep % 128 == 0
            return [(buf, dst, (slice(None), r, slice(None), pl.ds(c0, cstep)))
                    for r in range(nblk) for c0 in range(0, ncol, cstep)]

        def merge(*lists):
            keyed = [((n + 0.5) / len(l), k, d) for k, l in enumerate(lists) for n, d in enumerate(l)]
            return [d for _, _, d in sorted(keyed, key=lambda t: t[:2])]

        for buf, dst, idx in (merge(pieces(dw1_b, dw1_hbm), pieces(dw2_b, dw2_hbm))
                              + merge(pieces(dwq_b, dwq_hbm), pieces(dwo_b, dwo_hbm))):
            cp(buf.at[idx], dst.at[idx], sem_w).start()

        for src, dst in ((out_b, out_hbm), (dx_b, dx_hbm), (dgw_b, dgw_hbm), (dw1_b, dw1_hbm),
                         (dw2_b, dw2_hbm), (dwq_b, dwq_hbm), (dwo_b, dwo_hbm), (kbuf, dk_hbm), (vbuf, dv_hbm)):
            cp(src, dst, sem_w).wait()

    hbm = pl.BlockSpec(memory_space=pltpu.MemorySpace.HBM)
    sds = jax.ShapeDtypeStruct
    weights = (A_wq, A_wo, B_w1, B_w2)
    wrows = [max(8, WPIECE * 1024 // (w.shape[1] * 2) // 8 * 8) for w in weights]
    wsplit = [(WS, w.shape[0] // WS // n, n, w.shape[1]) for w, n in zip(weights, wrows)]
    assert all(w.shape[0] % (WS * n) == 0 for w, n in zip(weights, wrows))
    outs = pl.pallas_call(
        kernel,
        in_specs=[hbm] * 9,
        out_specs=[hbm] * 9,
        out_shape=[sds((B, D), bf16), sds((B, D), bf16), sds(kv_shape, bf16), sds(kv_shape, bf16)]
        + [sds(s, bf16) for s in wsplit] + [sds(gate_w.shape, bf16)],
        scratch_shapes=[pltpu.VMEM(kv_shape, bf16)] * 2
        + [pltpu.VMEM(w.shape, bf16) for w in weights]
        + [pltpu.VMEM(s, bf16) for s in wsplit]
        + [pltpu.VMEM((B, D), bf16), pltpu.VMEM((B, D), bf16), pltpu.VMEM((D,), bf16)] * 2
        + [pltpu.VMEM((16, HD), f32)] * 4
        + [pltpu.VMEM((8, SK), f32), pltpu.SemaphoreType.DMA(())],
        compiler_params=pltpu.CompilerParams(vmem_limit_bytes=110 * 1024 * 1024),
    )(A_x.reshape(B, D), A_k_cache.reshape(kv_shape), A_v_cache.reshape(kv_shape), A_wq, A_wo,
      B_w1, B_w2, gate_w, grad_out.reshape(B, D))
    return (outs[0].reshape(A_x.shape), outs[1].reshape(A_x.shape),
            outs[2].reshape(A_k_cache.shape), outs[3].reshape(A_v_cache.shape),
            *[o.reshape(w.shape) for o, w in zip(outs[4:8], weights)], outs[8])
```
